```python
import os as _os
_os.environ.setdefault("JAX_PLATFORMS", "cpu")
import jax
import jax.numpy as jnp

def _softmax(x, axis=-1):
    return jax.nn.softmax(x, axis=axis)
def _gelu(x):
    return jax.nn.gelu(x, approximate=True)
def _silu(x):
    return jax.nn.silu(x)
def _sigmoid(x):
    return jax.nn.sigmoid(x)
def _layernorm(x, axis=-1, eps=1e-5):
    m = jnp.mean(x, axis=axis, keepdims=True)
    v = jnp.var(x, axis=axis, keepdims=True)
    return (x - m) / jnp.sqrt(v + eps)
def _scatter_add(tgt, idx, src, axis=0):
    return tgt.at[idx].add(src)
def _segment_sum(src, seg, n):
    return jax.ops.segment_sum(src, seg, n)
class _Rng:
    def __init__(self, key):
        self._k = key
    def _next(self):
        self._k, sub = jax.random.split(self._k)
        return sub
    def normal(self, shape):
        return jax.random.normal(self._next(), shape, dtype=jnp.bfloat16)
    def randint(self, lo, hi, shape):
        return jax.random.randint(self._next(), shape, lo, hi, dtype=jnp.int32)
    def uniform(self, shape, lo=0.0, hi=1.0):
        return jax.random.uniform(self._next(), shape, jnp.bfloat16, lo, hi)
    def permutation(self, n):
        return jax.random.permutation(self._next(), n)


kernel_name = 'standalone__gqa_softmax__near_ridge'

def setup_inputs():
    _rng = _Rng(jax.random.key(int.from_bytes(__import__("os").urandom(4), "little")))
    _w = (lambda a: (lambda t: t.astype(jnp.bfloat16) if jnp.issubdtype(t.dtype, jnp.floating) else t)(jnp.asarray(a)))
    B, Hq, Hkv, Sq, Sk, D = 8, 16, 8, 160, 2048, 256
    return {
        "q": _w((lambda *s: _rng.normal(s) * 0.05)(B, Hq, Sq, D)),
        "k": _w((lambda *s: _rng.normal(s) * 3.2)(B, Hkv, Sk, D)),
        "v": _w((lambda *s: _rng.normal(s) * 0.05)(B, Hkv, Sk, D)),
    }

def reference(q, k, v):
    B, Hq, Sq, D = q.shape
    Hkv = k.shape[1]
    rep = Hq // Hkv
    k = jnp.repeat(k, rep, axis=1)
    v = jnp.repeat(v, rep, axis=1)
    scale = D ** -0.5
    scores = jnp.einsum("bhqd,bhkd->bhqk", q, k) * scale
    p = _softmax(scores, axis=-1)
    return jnp.einsum("bhqk,bhkd->bhqd", p, v)
```

```python
import functools

import jax
import jax.numpy as jnp
from jax import lax
import jax.experimental.pallas as pl
import jax.experimental.pallas.tpu as pltpu

NT = (((1,), (1,)), ((), ()))
LOG2E = 1.4426950408889634
F32 = jnp.float32
BF16 = jnp.bfloat16
LANES = 128


def _kernel(q_hbm, k_hbm, v_hbm, o_hbm,
            ub, ob, s_ref, m_ref, p0_ref, l0_ref, acc_ref,
            su, sk, so, sd,
            *, ND, TD, CH, NB, NO, NS, phases, K0C, scale, refill_at):
    H, M, D = q_hbm.shape
    SK = k_hbm.shape[1]
    NJ = SK // CH
    NL = CH // LANES
    C = scale * LOG2E
    OFF = 1

    starts = []
    u = NS
    for g, n in phases:
        assert g & (g - 1) == 0 and (u + OFF) % g == 0 or g == 1
        starts.append(u)
        u += g * n
    assert u == H - 1
    gmax = max(g for g, _ in phases)
    assert ND % 2 == 0 and TD + ND // 2 <= phases[-1][1]
    assert NB & (NB - 1) == 0 and NO & (NO - 1) == 0 and NB >= 2 * gmax and NO >= 2 * gmax and NS < NB

    def slot(w):
        return (w + OFF) & (NB - 1)

    def sem_idx(w):
        s = slot(w)
        if isinstance(w, (int)):
            g = 1
            for (gg, _), u0 in zip(phases, starts):
                if w >= u0:
                    g = gg
            return s & ~(g - 1)
        idx = s
        for (gg, _), u0 in zip(phases, starts):
            if gg > 1:
                idx = jnp.where(w >= u0, s & ~(gg - 1), idx)
        return idx

    def v_copy(w, sem):
        return pltpu.make_async_copy(v_hbm.at[w], ub.at[slot(w), pl.ds(0, SK)], sem)

    def k_copy(w, sem):
        return pltpu.make_async_copy(k_hbm.at[w + 1], ub.at[slot(w), pl.ds(SK, SK)], sem)

    def q_copy(w, sem):
        return pltpu.make_async_copy(q_hbm.at[w + 1], ub.at[slot(w), pl.ds(2 * SK, M)], sem)

    def o_copy(w):
        s = w & (NO - 1)
        return pltpu.make_async_copy(ob.at[s], o_hbm.at[w], so.at[s])

    def parked_copy(w, n):
        return pltpu.make_async_copy(ob.at[pl.ds(NO + w, n)], o_hbm.at[pl.ds(w, n)], sd.at[w // n if isinstance(w, int) else w >> 1])

    def wait_rows(ref, sem):
        pltpu.make_async_copy(ref, ref, sem).wait()

    def refill(w):
        sem = su.at[sem_idx(w)]

        @pl.when(w + 1 < H)
        def _():
            k_copy(w, sem).start()
            q_copy(w, sem).start()

        @pl.when(w < H)
        def _():
            v_copy(w, sem).start()

    def qk_tile(s, j):
        x = lax.dot_general(ub[s, pl.ds(2 * SK, M), :], ub[s, pl.ds(SK + j * CH, CH), :], NT,
                            preferred_element_type=F32)
        return x * C

    def lane_fold(op, run, x):
        for t in range(x.shape[1] // LANES):
            y = x[:, t * LANES:(t + 1) * LANES]
            run = y if run is None else op(run, y)
        return run

    def exp_tile(j, mb, lrun):
        p = jnp.exp2(s_ref[:, pl.ds(j * CH, CH)] - jnp.concatenate([mb] * NL, axis=1))
        return p.astype(BF16), lane_fold(jnp.add, lrun, p)

    def close_scores(mrun):
        mb = jnp.broadcast_to(jnp.max(mrun, axis=1, keepdims=True), (M, LANES))
        return (mb,) + exp_tile(0, mb, None)

    def scores_only(s, wait_chunk=None):
        mrun = None
        for j in range(NJ):
            if wait_chunk is not None:
                wait_chunk(j)
            x = qk_tile(s, j)
            mrun = lane_fold(jnp.maximum, mrun, x)
            s_ref[:, pl.ds(j * CH, CH)] = x
        return close_scores(mrun)

    def step(u, st, with_scores, hook=None, may_park=True):
        mb, p, lrun = st
        s = slot(u)
        acc = mrun = inv = None
        for j in range(NJ):
            if j > 0:
                p, lrun = exp_tile(j, mb, lrun)
            if j == NJ - 1:
                l = jnp.sum(lrun, axis=1, keepdims=True)
                r = pl.reciprocal(l, approx=True)
                inv = r + r * (1.0 - l * r)

            def scores():
                nonlocal mrun
                if with_scores:
                    x = qk_tile(s, j)
                    mrun = lane_fold(jnp.maximum, mrun, x)
                    s_ref[:, pl.ds(j * CH, CH)] = x

            if j > 0:
                scores()
            o = jnp.dot(p, ub[s, pl.ds(j * CH, CH), :], preferred_element_type=F32)
            if j == 0:
                acc_ref[...] = o
                acc = acc_ref[...]
                scores()
            else:
                acc = acc + o
            if hook is not None and j == refill_at:
                hook()
        res = (acc * inv).astype(ob.dtype)
        if isinstance(u, int) or may_park is False:
            ob[u & (NO - 1)] = res
            o_copy(u).start()
        else:
            ob[jnp.where(u < ND, NO + u, u & (NO - 1))] = res
            pl.when(u >= ND)(lambda: o_copy(u).start())
        return close_scores(mrun) if with_scores else None

    def save(st):
        m_ref[...], p0_ref[...], l0_ref[...] = st

    def restore():
        return m_ref[...], p0_ref[...], l0_ref[...]

    def wait_out(u):
        if isinstance(u, int):
            if u >= NO + ND:
                o_copy(u - NO).wait()
        else:
            pl.when(u >= NO + ND)(lambda: o_copy(u - NO).wait())

    s0 = slot(-1)
    KC = SK // K0C

    def k0_copy(c):
        return pltpu.make_async_copy(k_hbm.at[0, pl.ds(c * KC, KC)], ub.at[s0, pl.ds(SK + c * KC, KC)],
                                     sk.at[NS + 1 + c])

    q0_copy = pltpu.make_async_copy(q_hbm.at[0], ub.at[s0, pl.ds(2 * SK, M)], sk.at[NS])
    q0_copy.start()
    for c in range(K0C):
        k0_copy(c).start()
    for w in range(NB - 1):
        sem = su.at[sem_idx(w)]
        if w < NS:
            v_copy(w, sem).start()
            q_copy(w, sk.at[w]).start()
            k_copy(w, sk.at[w]).start()
        else:
            k_copy(w, sem).start()
            q_copy(w, sem).start()
            v_copy(w, sem).start()
    q0_copy.wait()
    save(scores_only(s0, lambda j: k0_copy(j * CH // KC).wait() if (j * CH) % KC == 0 else None))

    def split_body(u, carry):
        s = slot(u)
        wait_rows(ub.at[s, pl.ds(0, SK)], su.at[s])
        if NS > NO + ND:
            wait_out(u)
        step(u, restore(), False, hook=lambda: refill(u - 1 + NB))
        wait_rows(ub.at[s, pl.ds(SK, SK + M)], sk.at[u])
        save(scores_only(s))
        return carry

    if NS:
        lax.fori_loop(0, NS, split_body, 0)

    gprev = 1
    for (g, n), first in zip(phases, starts):
        def body(t, carry, g=g, first=first, gprev=gprev):
            u0 = first + t * g
            s = slot(u0)
            wait_rows(ub.at[pl.ds(s, g)], su.at[s])
            for i in range(g):
                if first >= NO + ND:
                    o_copy(u0 + i - NO).wait()
                else:
                    wait_out(u0 + i)

            def hook():
                for i in range(g):
                    w = u0 - g + i + NB
                    if i < g - gprev:
                        pl.when(t > 0)(functools.partial(refill, w))
                    else:
                        refill(w)
                if g == gmax and ND:
                    pl.when(jnp.logical_and(t >= TD, t < TD + ND // 2))(
                        lambda: parked_copy(2 * (t - TD), 2).start())

            st = restore()
            for i in range(g):
                st = step(u0 + i, st, True, hook=hook if i == 0 else None, may_park=first < ND)
            save(st)
            return carry

        if n:
            lax.fori_loop(0, n, body, 0)
            gprev = g

    u = H - 1
    wait_rows(ub.at[slot(u), pl.ds(0, SK)], su.at[sem_idx(u)])
    wait_out(u)
    step(u, restore(), False)
    for w in range(H - NO, H):
        o_copy(w).wait()
    for w in range(0, ND, 2):
        parked_copy(w, 2).wait()


def kern(q, k, v, CH=256, NB=16, NO=8, NS=2, N1=7, N2=7, N4=10, ND=16, TD=2, K0C=2, refill_at=1,
         vmem=100):
    B, Hq, Sq, D = q.shape
    Hkv, Sk = k.shape[1], k.shape[2]
    rep = Hq // Hkv
    H, M = B * Hkv, rep * Sq
    phases = tuple((g, n) for g, n in ((1, N1), (2, N2), (4, N4)) if n)
    q2 = q.reshape(H, M, D)
    k2 = k.reshape(H, Sk, D)
    v2 = v.reshape(H, Sk, D)
    any_spec = pl.BlockSpec(memory_space=pl.ANY)
    o = pl.pallas_call(
        functools.partial(_kernel, ND=ND, TD=TD, CH=CH, NB=NB, NO=NO, NS=NS, phases=phases, K0C=K0C,
                          scale=D ** -0.5, refill_at=refill_at),
        in_specs=[any_spec, any_spec, any_spec],
        out_specs=any_spec,
        out_shape=jax.ShapeDtypeStruct(q2.shape, q.dtype),
        scratch_shapes=[
            pltpu.VMEM((NB, 2 * Sk + M, D), BF16),
            pltpu.VMEM((NO + ND, M, D), q.dtype),
            pltpu.VMEM((M, Sk), F32),
            pltpu.VMEM((M, LANES), F32),
            pltpu.VMEM((M, CH), BF16),
            pltpu.VMEM((M, LANES), F32),
            pltpu.VMEM((M, D), F32),
            pltpu.SemaphoreType.DMA((NB,)),
            pltpu.SemaphoreType.DMA((NS + 1 + K0C,)),
            pltpu.SemaphoreType.DMA((NO,)),
            pltpu.SemaphoreType.DMA((max(ND // 2, 1),)),
        ],
        compiler_params=pltpu.CompilerParams(
            vmem_limit_bytes=vmem * 2**20,
            disable_bounds_checks=True,
            flags={"XLA_TPU_FORCE_LP_LLO_SCHEDULER": True},
        ),
    )(q2, k2, v2)
    return o.reshape(q.shape)


@jax.jit
def pallas_standalone__gqa_softmax__near_ridge_kernel(q: jax.Array, k: jax.Array, v: jax.Array):
    return kern(q, k, v)
```
